```python
import os as _os
_os.environ.setdefault("JAX_PLATFORMS", "cpu")
import jax
import jax.numpy as jnp

def _softmax(x, axis=-1):
    return jax.nn.softmax(x, axis=axis)
def _gelu(x):
    return jax.nn.gelu(x, approximate=True)
def _silu(x):
    return jax.nn.silu(x)
def _sigmoid(x):
    return jax.nn.sigmoid(x)
def _layernorm(x, axis=-1, eps=1e-5):
    m = jnp.mean(x, axis=axis, keepdims=True)
    v = jnp.var(x, axis=axis, keepdims=True)
    return (x - m) / jnp.sqrt(v + eps)
def _scatter_add(tgt, idx, src, axis=0):
    return tgt.at[idx].add(src)
def _segment_sum(src, seg, n):
    return jax.ops.segment_sum(src, seg, n)
class _Rng:
    def __init__(self, key):
        self._k = key
    def _next(self):
        self._k, sub = jax.random.split(self._k)
        return sub
    def normal(self, shape):
        return jax.random.normal(self._next(), shape, dtype=jnp.bfloat16)
    def randint(self, lo, hi, shape):
        return jax.random.randint(self._next(), shape, lo, hi, dtype=jnp.int32)
    def uniform(self, shape, lo=0.0, hi=1.0):
        return jax.random.uniform(self._next(), shape, jnp.bfloat16, lo, hi)
    def permutation(self, n):
        return jax.random.permutation(self._next(), n)


kernel_name = 'concat_heads__sliding_block_cached__sliding_block_cached__decode'

def setup_inputs():
    _rng = _Rng(jax.random.key(int.from_bytes(__import__("os").urandom(4), "little")))
    _w = (lambda a: (lambda t: t.astype(jnp.bfloat16) if jnp.issubdtype(t.dtype, jnp.floating) else t)(jnp.asarray(a)))
    def _A_setup():
        B, Sq, D = 2, 1, 640
        Hq, Hkv, Sk, Dh = 32, 32, 4096, 128
        assert Hq % Hkv == 0, (Hq, Hkv)
        return {
            "x": _w((lambda *s: _rng.normal(s) * 0.8)(B, Sq, D)),
            "k_cache": _w((lambda *s: _rng.normal(s) * 0.8)(B, Hkv, Sk, Dh)),
            "v_cache": _w((lambda *s: _rng.normal(s) * 0.05)(B, Hkv, Sk, Dh)),
            "wq": _w((lambda *s: _rng.normal(s) * 0.8)(D, Hq * Dh) * (D ** -0.5)),
            "wo": _w((lambda *s: _rng.normal(s) * 0.05)(Hq * Dh, D) * ((Hq * Dh) ** -0.5)),
        }
    _A_in = _A_setup()

    def _B_setup():
        B, Sq, D = 2, 1, 640
        Hq, Hkv, Sk, Dh = 32, 32, 4096, 128
        assert Hq % Hkv == 0, (Hq, Hkv)
        return {
            "x": _w((lambda *s: _rng.normal(s) * 0.8)(B, Sq, D)),
            "k_cache": _w((lambda *s: _rng.normal(s) * 0.8)(B, Hkv, Sk, Dh)),
            "v_cache": _w((lambda *s: _rng.normal(s) * 0.05)(B, Hkv, Sk, Dh)),
            "wq": _w((lambda *s: _rng.normal(s) * 0.8)(D, Hq * Dh) * (D ** -0.5)),
            "wo": _w((lambda *s: _rng.normal(s) * 0.05)(Hq * Dh, D) * ((Hq * Dh) ** -0.5)),
        }
    _B_in = _B_setup()

    return {
        "A_x": _A_in["x"],
        "A_k_cache": _A_in["k_cache"],
        "A_v_cache": _A_in["v_cache"],
        "A_wq": _A_in["wq"],
        "A_wo": _A_in["wo"],
        "B_x": _B_in["x"],
        "B_k_cache": _B_in["k_cache"],
        "B_v_cache": _B_in["v_cache"],
        "B_wq": _B_in["wq"],
        "B_wo": _B_in["wo"],
    }

def reference(A_x, A_k_cache, A_v_cache, A_wq, A_wo, B_x, B_k_cache, B_v_cache, B_wq, B_wo):
    def _A_ref(x, k_cache, v_cache, wq, wo):
        B, Sq, D = x.shape
        Hq, Dh = 32, 128
        Hkv, Sk = k_cache.shape[1], k_cache.shape[2]
        W = min(4096, max(256, Sk // 4))
        rep = Hq // Hkv
        q = (lambda x, *d: x.transpose(*d))((x @ wq).reshape(B, Sq, Hq, Dh), 0, 2, 1, 3)
        k = jnp.repeat(k_cache[:, :, Sk - W:, :], rep, axis=1)
        v = jnp.repeat(v_cache[:, :, Sk - W:, :], rep, axis=1)
        scores = jnp.einsum("bhqd,bhkd->bhqk", q, k) * (Dh ** -0.5)
        p = _softmax(scores, axis=-1)
        o = jnp.einsum("bhqk,bhkd->bhqd", p, v)
        return (lambda x, *d: x.transpose(*d))(o, 0, 2, 1, 3).reshape(B, Sq, Hq * Dh) @ wo

    def _B_ref(x, k_cache, v_cache, wq, wo):
        B, Sq, D = x.shape
        Hq, Dh = 32, 128
        Hkv, Sk = k_cache.shape[1], k_cache.shape[2]
        W = min(4096, max(256, Sk // 4))
        rep = Hq // Hkv
        q = (lambda x, *d: x.transpose(*d))((x @ wq).reshape(B, Sq, Hq, Dh), 0, 2, 1, 3)
        k = jnp.repeat(k_cache[:, :, Sk - W:, :], rep, axis=1)
        v = jnp.repeat(v_cache[:, :, Sk - W:, :], rep, axis=1)
        scores = jnp.einsum("bhqd,bhkd->bhqk", q, k) * (Dh ** -0.5)
        p = _softmax(scores, axis=-1)
        o = jnp.einsum("bhqk,bhkd->bhqd", p, v)
        return (lambda x, *d: x.transpose(*d))(o, 0, 2, 1, 3).reshape(B, Sq, Hq * Dh) @ wo

    a = _A_ref(A_x, A_k_cache, A_v_cache, A_wq, A_wo)
    b = _B_ref(B_x, B_k_cache, B_v_cache, B_wq, B_wo)
    return jnp.concatenate([a, b], axis=-1)
```

```python
import functools

import jax
import jax.numpy as jnp
import jax.experimental.pallas as pl
import jax.experimental.pallas.tpu as pltpu

_HQ, _DH = 32, 128
_HG = 2


def _branch_step(x_ref, k_ref, v_ref, wq_ref, wo_ref, acc_ref, step):
    B = x_ref.shape[0]
    hg = k_ref.shape[1]
    x = x_ref[...]
    q = jnp.dot(x, wq_ref[...], preferred_element_type=jnp.float32).astype(jnp.bfloat16)
    row = jax.lax.broadcasted_iota(jnp.int32, (8, _DH), 0)
    o_cols = []
    for h in range(hg):
        o_h = jnp.zeros((8, _DH), jnp.float32)
        for b in range(B):
            qr = jnp.broadcast_to(q[b:b + 1, h * _DH:(h + 1) * _DH], (8, _DH))
            s = jax.lax.dot_general(qr, k_ref[b, h], (((1,), (1,)), ((), ())),
                                    preferred_element_type=jnp.float32) * (_DH ** -0.5)
            m = jnp.max(s, axis=-1, keepdims=True)
            e = jnp.exp(s - m)
            p = e / jnp.sum(e, axis=-1, keepdims=True)
            o = jnp.dot(p.astype(jnp.bfloat16), v_ref[b, h], preferred_element_type=jnp.float32)
            o_h = jnp.where(row == b, o, o_h)
        o_cols.append(o_h)
    o_all = jnp.concatenate(o_cols, axis=1).astype(jnp.bfloat16)
    part = jnp.dot(o_all, wo_ref[...], preferred_element_type=jnp.float32)

    @pl.when(step == 0)
    def _():
        acc_ref[...] = part

    @pl.when(step > 0)
    def _():
        acc_ref[...] += part


def _kernel(ax, ak, av, awq, awo, bx, bk, bv, bwq, bwo, out_ref, acc_a, acc_b):
    step = pl.program_id(0)
    _branch_step(ax, ak, av, awq, awo, acc_a, step)
    _branch_step(bx, bk, bv, bwq, bwo, acc_b, step)
    B, D = ax.shape

    @pl.when(step == pl.num_programs(0) - 1)
    def _():
        out_ref[:, :D] = acc_a[0:B, :].astype(out_ref.dtype)
        out_ref[:, D:] = acc_b[0:B, :].astype(out_ref.dtype)


@jax.jit
def pallas_concat_heads__sliding_block_cached__sliding_block_cached__decode_kernel(
    A_x: jax.Array,
    A_k_cache: jax.Array,
    A_v_cache: jax.Array,
    A_wq: jax.Array,
    A_wo: jax.Array,
    B_x: jax.Array,
    B_k_cache: jax.Array,
    B_v_cache: jax.Array,
    B_wq: jax.Array,
    B_wo: jax.Array,
):
    B, Sq, D = A_x.shape
    Sk = A_k_cache.shape[2]
    W = min(4096, max(256, Sk // 4))
    assert Sq == 1 and Sk % W == 0
    wblk = Sk // W - 1
    hg = _HG
    x_spec = pl.BlockSpec((B, D), lambda i: (0, 0))
    kv_spec = pl.BlockSpec((B, hg, W, _DH), lambda i: (0, i, wblk, 0))
    wq_spec = pl.BlockSpec((D, hg * _DH), lambda i: (0, i))
    wo_spec = pl.BlockSpec((hg * _DH, D), lambda i: (i, 0))
    out = pl.pallas_call(
        _kernel,
        grid=(_HQ // hg,),
        in_specs=[x_spec, kv_spec, kv_spec, wq_spec, wo_spec] * 2,
        out_specs=pl.BlockSpec((B, 2 * D), lambda i: (0, 0)),
        out_shape=jax.ShapeDtypeStruct((B, 2 * D), A_x.dtype),
        scratch_shapes=[pltpu.VMEM((8, D), jnp.float32), pltpu.VMEM((8, D), jnp.float32)],
        compiler_params=pltpu.CompilerParams(
            dimension_semantics=("arbitrary",), vmem_limit_bytes=64 * 1024 * 1024),
    )(A_x.reshape(B, D), A_k_cache, A_v_cache, A_wq, A_wo,
      B_x.reshape(B, D), B_k_cache, B_v_cache, B_wq, B_wo)
    return out.reshape(B, Sq, 2 * D)
```

```python
import jax
import jax.numpy as jnp
import jax.experimental.pallas as pl
import jax.experimental.pallas.tpu as pltpu

_HQ, _DH = 32, 128
_HC = 8
_NC = _HQ // _HC
_H_UNROLL = 2
_Q_COLS = 512
_WO_UNROLL = 4
_WO_SPLITS = ((4096,), (1024, 1024, 1024, 512, 256, 128, 128))

_S_X, _S_WQ, _S_KV = 0, 2, 4
_S_WO = _S_KV + 4 * _NC
_S_OUT = _S_WO + len(_WO_SPLITS[0]) + len(_WO_SPLITS[1])
_NUM_SEMS = _S_OUT + 1


def _kernel(ax, ak, av, awq, awo, bx, bk, bv, bwq, bwo, out_hbm,
            xa_buf, xb_buf, wq_buf, wo_buf, k_buf, v_buf, q_scr, o_scr, out_buf):
    B, D = ax.shape
    Sk = ak.shape[2]
    W = k_buf.shape[-2]
    branches = ((ax, ak, av, awq, awo, xa_buf), (bx, bk, bv, bwq, bwo, xb_buf))

    def body(sems):
        def x_copy(br):
            return pltpu.make_async_copy(branches[br][0], branches[br][5], sems.at[_S_X + br])

        def wq_copy(br):
            return pltpu.make_async_copy(branches[br][3], wq_buf.at[br], sems.at[_S_WQ + br])

        def k_copy(br, c):
            return pltpu.make_async_copy(
                branches[br][1].at[:, pl.ds(c * _HC, _HC), pl.ds(Sk - W, W), :],
                k_buf.at[br, c], sems.at[_S_KV + br * 2 * _NC + c])

        def v_copy(br, c):
            return pltpu.make_async_copy(
                branches[br][2].at[:, pl.ds(c * _HC, _HC), pl.ds(Sk - W, W), :],
                v_buf.at[br, c], sems.at[_S_KV + br * 2 * _NC + _NC + c])

        def wo_copy(br, i):
            off, n = sum(_WO_SPLITS[br][:i]), _WO_SPLITS[br][i]
            sem = _S_WO + (len(_WO_SPLITS[0]) if br else 0) + i
            return pltpu.make_async_copy(
                branches[br][4].at[pl.ds(off, n), :], wo_buf.at[br, pl.ds(off, n), :], sems.at[sem])

        for br in range(2):
            x_copy(br).start()
            wq_copy(br).start()
            for c in range(_NC):
                k_copy(br, c).start()
                v_copy(br, c).start()
            for i in range(len(_WO_SPLITS[br])):
                wo_copy(br, i).start()

        row_h = jax.lax.broadcasted_iota(jnp.int32, (8, _DH), 0)
        row_x = jax.lax.broadcasted_iota(jnp.int32, (8, D), 0)

        for br in range(2):
            x_copy(br).wait()
            xv = branches[br][5][...].astype(jnp.float32)
            x8 = jnp.zeros((8, D), jnp.float32)
            for b in range(B):
                x8 = jnp.where(row_x == b, jnp.broadcast_to(xv[b:b + 1], (8, D)), x8)
            x8 = x8.astype(jnp.bfloat16)
            wq_copy(br).wait()

            def q_body(c, carry, br=br, x8=x8):
                off = pl.multiple_of(c * _Q_COLS, _Q_COLS)
                r = jnp.dot(x8, wq_buf[br, :, pl.ds(off, _Q_COLS)],
                            preferred_element_type=jnp.float32)
                for j in range(_Q_COLS // _DH):
                    q_scr[c * (_Q_COLS // _DH) + j] = r[:, j * _DH:(j + 1) * _DH]
                return carry

            jax.lax.fori_loop(0, (_HQ * _DH) // _Q_COLS, q_body, 0)

            def chunk_body(c, carry, br=br):
                k_copy(br, c).wait()
                v_copy(br, c).wait()

                def head_body(i, carry):
                    for u in range(_H_UNROLL):
                        hh = i * _H_UNROLL + u
                        h = c * _HC + hh
                        q = q_scr[h].astype(jnp.bfloat16)
                        oh = jnp.zeros((8, _DH), jnp.float32)
                        for b in range(B):
                            s = jax.lax.dot_general(
                                q, k_buf[br, c, b, hh], (((1,), (1,)), ((), ())),
                                preferred_element_type=jnp.float32) * (_DH ** -0.5)
                            m = jnp.max(s, axis=-1, keepdims=True)
                            e = jnp.exp(s - m)
                            denom = jnp.sum(e, axis=-1, keepdims=True)
                            o = jnp.dot(e.astype(jnp.bfloat16), v_buf[br, c, b, hh],
                                        preferred_element_type=jnp.float32) / denom
                            oh = jnp.where(row_h == b, o, oh)
                        o_scr[h] = oh
                    return carry

                jax.lax.fori_loop(0, _HC // _H_UNROLL, head_body, 0)
                return carry

            jax.lax.fori_loop(0, _NC, chunk_body, 0)

            acc = jnp.zeros((8, D), jnp.float32)
            for i, n in enumerate(_WO_SPLITS[br]):
                wo_copy(br, i).wait()
                h0 = sum(_WO_SPLITS[br][:i]) // _DH
                nh = n // _DH
                un = max(d for d in range(1, _WO_UNROLL + 1) if nh % d == 0)

                def wo_body(t, acc, br=br, h0=h0, un=un):
                    for u in range(un):
                        h = h0 + t * un + u
                        rows = pl.ds(pl.multiple_of(h * _DH, _DH), _DH)
                        acc = acc + jnp.dot(o_scr[h].astype(jnp.bfloat16), wo_buf[br, rows, :],
                                            preferred_element_type=jnp.float32)
                    return acc

                if nh == un:
                    acc = wo_body(0, acc)
                else:
                    acc = jax.lax.fori_loop(0, nh // un, wo_body, acc)
            out_buf[:, br * D:(br + 1) * D] = acc[0:B, :].astype(out_buf.dtype)

        out_copy = pltpu.make_async_copy(out_buf, out_hbm, sems.at[_S_OUT])
        out_copy.start()
        out_copy.wait()

    pl.run_scoped(body, pltpu.SemaphoreType.DMA((_NUM_SEMS,)))


@jax.jit
def pallas_concat_heads__sliding_block_cached__sliding_block_cached__decode_kernel(
    A_x: jax.Array,
    A_k_cache: jax.Array,
    A_v_cache: jax.Array,
    A_wq: jax.Array,
    A_wo: jax.Array,
    B_x: jax.Array,
    B_k_cache: jax.Array,
    B_v_cache: jax.Array,
    B_wq: jax.Array,
    B_wo: jax.Array,
):
    B, Sq, D = A_x.shape
    Hkv, Sk, Dh = A_k_cache.shape[1:]
    assert Sq == 1 and B <= 8 and Hkv == _HQ and Dh == _DH
    W = min(4096, max(256, Sk // 4))
    dt = A_x.dtype

    out = pl.pallas_call(
        _kernel,
        in_specs=[pl.BlockSpec(memory_space=pl.ANY)] * 10,
        out_specs=pl.BlockSpec(memory_space=pl.ANY),
        out_shape=jax.ShapeDtypeStruct((B, 2 * D), dt),
        scratch_shapes=[
            pltpu.VMEM((B, D), dt),
            pltpu.VMEM((B, D), dt),
            pltpu.VMEM((2, D, _HQ * _DH), dt),
            pltpu.VMEM((2, _HQ * _DH, D), dt),
            pltpu.VMEM((2, _NC, B, _HC, W, _DH), dt),
            pltpu.VMEM((2, _NC, B, _HC, W, _DH), dt),
            pltpu.VMEM((_HQ, 8, _DH), jnp.float32),
            pltpu.VMEM((_HQ, 8, _DH), jnp.float32),
            pltpu.VMEM((B, 2 * D), dt),
        ],
        compiler_params=pltpu.CompilerParams(vmem_limit_bytes=110 * 1024 * 1024),
    )(A_x.reshape(B, D), A_k_cache, A_v_cache, A_wq, A_wo,
      B_x.reshape(B, D), B_k_cache, B_v_cache, B_wq, B_wo)
    return out.reshape(B, Sq, 2 * D)
```
